```python
import jax
import jax.numpy as jnp

def _softmax(x, axis=-1):
    return jax.nn.softmax(x, axis=axis)
def _gelu(x):
    return jax.nn.gelu(x, approximate=True)
def _silu(x):
    return jax.nn.silu(x)
def _sigmoid(x):
    return jax.nn.sigmoid(x)
def _layernorm(x, axis=-1, eps=1e-5):
    m = jnp.mean(x, axis=axis, keepdims=True)
    v = jnp.var(x, axis=axis, keepdims=True)
    return (x - m) / jnp.sqrt(v + eps)
def _scatter_add(tgt, idx, src, axis=0):
    return tgt.at[idx].add(src)
def _segment_sum(src, seg, n):
    return jax.ops.segment_sum(src, seg, n)
class _Rng:
    def __init__(self, key):
        self._k = key
    def _next(self):
        self._k, sub = jax.random.split(self._k)
        return sub
    def normal(self, shape):
        return jax.random.normal(self._next(), shape, dtype=jnp.bfloat16)
    def randint(self, lo, hi, shape):
        return jax.random.randint(self._next(), shape, lo, hi, dtype=jnp.int32)
    def uniform(self, shape, lo=0.0, hi=1.0):
        return jax.random.uniform(self._next(), shape, jnp.bfloat16, lo, hi)
    def permutation(self, n):
        return jax.random.permutation(self._next(), n)


kernel_name = 'standalone__modern_conv_block_replknet__vision'

def setup_inputs():
    _rng = _Rng(jax.random.key(int.from_bytes(__import__("os").urandom(4), "little")))
    _w = (lambda a: (lambda t: t.astype(jnp.bfloat16) if jnp.issubdtype(t.dtype, jnp.floating) else t)(jnp.asarray(a)))
    H = W = 512
    C = 96
    K = 3
    return {
        "x": _w((lambda *s: _rng.normal(s) * 0.05)(1, H, W, C)),
        "dw_large": _w((lambda *s: _rng.normal(s) * 0.05)(K, K, C) * (1.0 / K)),
        "dw_small": _w((lambda *s: _rng.normal(s) * 0.05)(5, 5, C) * 0.2),
        "w1": _w((lambda *s: _rng.normal(s) * 0.05)(C, 4 * C) * (C ** -0.5)),
        "w2": _w((lambda *s: _rng.normal(s) * 0.05)(4 * C, C) * ((4 * C) ** -0.5)),
    }

def reference(x, dw_large, dw_small, w1, w2):
    B, H, W, C = x.shape
    Kl = dw_large.shape[0]
    pl = (Kl - 1) // 2
    xpl = jnp.pad(x, ((0,0),(pl,pl),(pl,pl),(0,0)))
    out = jnp.zeros_like(x)
    for i in range(Kl):
        for j in range(Kl):
            out = out + xpl[:, i:i+H, j:j+W, :] * dw_large[i, j][None, None, None, :]
    Ks = dw_small.shape[0]
    ps = (Ks - 1) // 2
    xps = jnp.pad(x, ((0,0),(ps,ps),(ps,ps),(0,0)))
    for i in range(Ks):
        for j in range(Ks):
            out = out + xps[:, i:i+H, j:j+W, :] * dw_small[i, j][None, None, None, :]
    h = _layernorm(out, axis=-1)
    h = _gelu(jnp.einsum('bhwc,ce->bhwe', h, w1))
    h = jnp.einsum('bhwe,ec->bhwc', h, w2)
    return x + h
```

```python
import functools
import math

import jax
import jax.numpy as jnp
import jax.experimental.pallas as pl
import jax.experimental.pallas.tpu as pltpu

TH = 8
R = 2
NS = 16
L = 128
RG = 1
MD = 2
XP = 1
LA = 6
MCH = 384
NT = 256

_C1 = math.sqrt(2.0 / math.pi)
_S = (_C1 * 0.044715) ** (1.0 / 3.0)
_KK = _C1 / _S
_OUT = 0.5 / _S


def _kernel(x_ref, dl_ref, ds_ref, w1_ref, w2t_ref, o_ref,
            ring, wb, w1t, w2t, hn, tmp, *, C, W, E, K, Kl, Ks):
    s = pl.program_id(0)
    ns = pl.num_programs(0)
    P = K // 2
    T = W // L
    CB = C // 8
    f32, bf16, u32 = jnp.float32, jnp.bfloat16, jnp.uint32

    @pl.when(s == 0)
    def _init():
        w1t[...] = pltpu.bitcast(w1_ref[...].astype(f32).T.astype(bf16), u32)
        w2t[...] = pltpu.bitcast(w2t_ref[...], u32)
        offs = (K - Ks) // 2
        offl = (K - Kl) // 2
        for i in range(K):
            for j in range(K):
                v = jnp.zeros((1, C), f32)
                if 0 <= i - offs < Ks and 0 <= j - offs < Ks:
                    v = v + ds_ref[i - offs, pl.ds(j - offs, 1), :].astype(f32)
                if 0 <= i - offl < Kl and 0 <= j - offl < Kl:
                    v = v + dl_ref[i - offl, pl.ds(j - offl, 1), :].astype(f32)
                wb[i * K + j] = jnp.broadcast_to(v, (L, C)).T

        def z(k, c):
            ring[k] = jnp.zeros((C, W), f32)
            return c
        jax.lax.fori_loop(0, NS, z, 0)
        hn[...] = jnp.zeros(hn.shape, hn.dtype)

    lane = jax.lax.broadcasted_iota(jnp.int32, (8, L), 1)

    def stage_a(m, r):
        row = m * R + r
        ring[(s * TH + row) & (NS - 1)] = x_ref[row].astype(f32)

    def stage_b(m, cb, gen):
        cs = pl.ds(cb * 8, 8)
        base = (s - 1) * TH + m * R + R - P + NS
        slots = [(base + q) & (NS - 1) for q in range(R + K - 1)]
        for r0 in range(0, R, RG):
            acc, pend = {}, None
            for j in [j for j in range(K) if j != P] + [P]:
                wv = [wb[i * K + j, cs, :] for i in range(K)]
                ps = {}
                for t in range(T):
                    for q in range(r0, r0 + RG + K - 1):
                        v = ring[slots[q], cs, pl.ds(t * L, L)]
                        for r in range(r0, r0 + RG):
                            i = q - r
                            if 0 <= i < K:
                                p = v * wv[i]
                                ps[r, t] = ps[r, t] + p if (r, t) in ps else p
                    if j != P:
                        for r in range(r0, r0 + RG):
                            ps[r, t] = pltpu.roll(ps[r, t], (P - j) % L, 1)
                    if r0 == 0:
                        next(gen, None)
                        if t < XP:
                            next(gen, None)
                for item in (pend, (j, ps) if j == P else None):
                    if item is None:
                        continue
                    d, pp = item[0] - P, item[1]
                    for (r, t), val in pp.items():
                        if d > 0:
                            val = jnp.where(lane < L - d, val, pp.get((r, t + 1), 0.0))
                        elif d < 0:
                            val = jnp.where(lane >= -d, val, pp.get((r, t - 1), 0.0))
                        acc[r, t] = acc[r, t] + val if (r, t) in acc else val
                pend = (j, ps)
            for (r, t), a in acc.items():
                tmp[r, cs, pl.ds(t * L, L)] = a

    def stage_ln(m, r, t):
        ts = pl.ds(t * L, L)
        v = tmp[r, :, ts]
        mean = jnp.sum(v, axis=0, keepdims=True) * (1.0 / C)
        d = v - mean
        var = jnp.sum(d * d, axis=0, keepdims=True) * (1.0 / C)
        sc = jax.lax.rsqrt(var + 1e-5) * _S
        hn[r, :, ts] = pltpu.bitcast((d * sc).astype(bf16), u32)

    def stage_c(m):
        units = [(r, t, e) for r in range(R) for t in range(T) for e in range(E // L)]

        def mm1(r, t, e):
            h = pltpu.bitcast(hn[r, :, pl.ds(t * L, L)], bf16)
            w = pltpu.bitcast(w1t[pl.ds(e * L // 2, L // 2), :], bf16)
            return jnp.dot(w, h, preferred_element_type=f32)

        def fin(r, t, os):
            row = m * R + r
            slot = ((s - 1) * TH + row + NS) & (NS - 1)
            ts = pl.ds(t * L, L)
            acc = sum(os[1:], os[0])
            o_ref[row, :, ts] = (ring[slot, :, ts] + acc * _OUT).astype(o_ref.dtype)

        q = [mm1(*u) for u in units[:LA]]
        os, gq = [], []

        def mm2(r, t, e, g):
            w = pltpu.bitcast(w2t[:, pl.ds(e * L, L)], bf16)
            os.append(jnp.dot(w, g, preferred_element_type=f32))
            if e == E // L - 1:
                fin(r, t, os)
                os.clear()

        for n, (r, t, e) in enumerate(units):
            if n + LA < len(units):
                q.append(mm1(*units[n + LA]))
            yield
            bb = q.pop(0)
            gs = []
            for k in range(L // 16):
                b = bb[k * 16:(k + 1) * 16]
                th = jnp.tanh(b * (b * b + _KK))
                gs.append(b * th + b)
                yield
            gq.append((r, t, e, jnp.concatenate(gs, 0).astype(bf16)))
            if len(gq) > MD:
                mm2(*gq.pop(0))
            yield
        for u in gq:
            mm2(*u)

    def body(m, c):
        @pl.when(jnp.logical_and(s == ns - 1, m == 1))
        def _():
            for r in range(P):
                slot = (s * TH + r) & (NS - 1)
                ring[slot] = jnp.zeros((C, W), f32)

        gen = stage_c(m)
        next(gen)
        for r in range(R):
            stage_a(m, r)
        for cb in range(CB):
            stage_b(m, cb, gen)
        for _ in gen:
            pass
        for r in range(R):
            for t in range(T):
                stage_ln(m, r, t)
        return c

    jax.lax.fori_loop(0, TH // R, body, 0)


@jax.jit
def pallas_standalone__modern_conv_block_replknet__vision_kernel(
    x: jax.Array,
    dw_large: jax.Array,
    dw_small: jax.Array,
    w1: jax.Array,
    w2: jax.Array,
):
    B, H, W, C = x.shape
    E = w1.shape[1]
    Kl, Ks = dw_large.shape[0], dw_small.shape[0]
    K = max(Kl, Ks)
    assert B == 1 and K <= 5 and H % TH == 0 and W % L == 0 and C % 16 == 0
    nb = H // TH
    xt = jnp.transpose(x.reshape(H, W, C), (0, 2, 1))
    full = lambda a: pl.BlockSpec(a.shape, lambda s: (0,) * a.ndim)
    w2t = w2.T
    out = pl.pallas_call(
        functools.partial(_kernel, C=C, W=W, E=E, K=K, Kl=Kl, Ks=Ks),
        grid=(nb + 1,),
        in_specs=[
            pl.BlockSpec((TH, C, W), lambda s: (jnp.minimum(s, nb - 1), 0, 0)),
            full(dw_large), full(dw_small), full(w1), full(w2t),
        ],
        out_specs=pl.BlockSpec((TH, C, W), lambda s: (jnp.maximum(s - 1, 0), 0, 0)),
        out_shape=jax.ShapeDtypeStruct((H, C, W), x.dtype),
        scratch_shapes=[
            pltpu.VMEM((NS, C, W), jnp.float32),
            pltpu.VMEM((K * K, C, L), jnp.float32),
            pltpu.VMEM((E // 2, C), jnp.uint32),
            pltpu.VMEM((C // 2, E), jnp.uint32),
            pltpu.VMEM((R, C // 2, W), jnp.uint32),
            pltpu.VMEM((R, C, W), jnp.float32),
        ],
        compiler_params=pltpu.CompilerParams(
            dimension_semantics=("arbitrary",),
            vmem_limit_bytes=64 * 1024 * 1024,
        ),
    )(xt, dw_large, dw_small, w1, w2t)
    return jnp.transpose(out, (0, 2, 1)).reshape(B, H, W, C)
```

```python
import functools
import math

import jax
import jax.numpy as jnp
import jax.experimental.pallas as pl
import jax.experimental.pallas.tpu as pltpu

TH = 8
R = 4
NS = 32
L = 128
RG = 1
MD = 2
XP = 1
LA = 6
MCH = 384
NT = 256

_C1 = math.sqrt(2.0 / math.pi)
_S = (_C1 * 0.044715) ** (1.0 / 3.0)
_KK = _C1 / _S
_OUT = 0.5 / _S


def _kernel(x_ref, dl_ref, ds_ref, w1_ref, w2t_ref, o_ref,
            ring, wb, w1t, w2t, hn, tmp, *, C, W, E, K, Kl, Ks):
    s = pl.program_id(0)
    ns = pl.num_programs(0)
    P = K // 2
    T = W // L
    CB = C // 8
    f32, bf16, u32 = jnp.float32, jnp.bfloat16, jnp.uint32

    @pl.when(s == 0)
    def _init():
        w1t[...] = pltpu.bitcast(w1_ref[...].astype(f32).T.astype(bf16), u32)
        w2t[...] = pltpu.bitcast(w2t_ref[...], u32)
        offs = (K - Ks) // 2
        offl = (K - Kl) // 2
        for i in range(K):
            for j in range(K):
                v = jnp.zeros((1, C), f32)
                if 0 <= i - offs < Ks and 0 <= j - offs < Ks:
                    v = v + ds_ref[i - offs, pl.ds(j - offs, 1), :].astype(f32)
                if 0 <= i - offl < Kl and 0 <= j - offl < Kl:
                    v = v + dl_ref[i - offl, pl.ds(j - offl, 1), :].astype(f32)
                wb[i * K + j] = jnp.broadcast_to(v, (L, C)).T

        def z(k, c):
            ring[k] = jnp.zeros((C, W), f32)
            return c
        jax.lax.fori_loop(0, NS, z, 0)
        hn[...] = jnp.zeros(hn.shape, hn.dtype)

    lane = jax.lax.broadcasted_iota(jnp.int32, (8, L), 1)

    def stage_a(m, r):
        row = m * R + r
        ring[(s * TH + row) & (NS - 1)] = jnp.where(
            s == ns - 1, 0.0, x_ref[row].astype(f32))

    def stage_b(m, cb, gen):
        cs = pl.ds(cb * 8, 8)
        base = (s - 1) * TH + m * R + R - P + NS
        slots = [(base + q) & (NS - 1) for q in range(R + K - 1)]
        for r0 in range(0, R, RG):
            acc, pend = {}, None
            for j in [j for j in range(K) if j != P] + [P]:
                wv = [wb[i * K + j, cs, :] for i in range(K)]
                ps = {}
                for t in range(T):
                    for q in range(r0, r0 + RG + K - 1):
                        v = ring[slots[q], cs, pl.ds(t * L, L)]
                        for r in range(r0, r0 + RG):
                            i = q - r
                            if 0 <= i < K:
                                p = v * wv[i]
                                ps[r, t] = ps[r, t] + p if (r, t) in ps else p
                    if j != P:
                        for r in range(r0, r0 + RG):
                            ps[r, t] = pltpu.roll(ps[r, t], (P - j) % L, 1)
                    if r0 == 0:
                        next(gen, None)
                        if t < XP:
                            next(gen, None)
                for item in (pend, (j, ps) if j == P else None):
                    if item is None:
                        continue
                    d, pp = item[0] - P, item[1]
                    for (r, t), val in pp.items():
                        if d > 0:
                            val = jnp.where(lane < L - d, val, pp.get((r, t + 1), 0.0))
                        elif d < 0:
                            val = jnp.where(lane >= -d, val, pp.get((r, t - 1), 0.0))
                        acc[r, t] = acc[r, t] + val if (r, t) in acc else val
                pend = (j, ps)
            for (r, t), a in acc.items():
                tmp[r, cs, pl.ds(t * L, L)] = a

    def stage_ln(m, r, t):
        ts = pl.ds(t * L, L)
        v = tmp[r, :, ts]
        mean = jnp.sum(v, axis=0, keepdims=True) * (1.0 / C)
        d = v - mean
        var = jnp.sum(d * d, axis=0, keepdims=True) * (1.0 / C)
        sc = jax.lax.rsqrt(var + 1e-5) * _S
        hn[r, :, ts] = pltpu.bitcast((d * sc).astype(bf16), u32)

    def stage_c(m):
        units = [(r, t, e) for r in range(R) for t in range(T) for e in range(E // L)]

        def mm1(r, t, e):
            h = pltpu.bitcast(hn[r, :, pl.ds(t * L, L)], bf16)
            w = pltpu.bitcast(w1t[pl.ds(e * L // 2, L // 2), :], bf16)
            return jnp.dot(w, h, preferred_element_type=f32)

        def fin(r, t, os):
            row = m * R + r
            slot = ((s - 1) * TH + row + NS) & (NS - 1)
            ts = pl.ds(t * L, L)
            acc = sum(os[1:], os[0])
            o_ref[row, :, ts] = (ring[slot, :, ts] + acc * _OUT).astype(o_ref.dtype)

        q = [mm1(*u) for u in units[:LA]]
        os, gq = [], []

        def mm2(r, t, e, g):
            w = pltpu.bitcast(w2t[:, pl.ds(e * L, L)], bf16)
            os.append(jnp.dot(w, g, preferred_element_type=f32))
            if e == E // L - 1:
                fin(r, t, os)
                os.clear()

        for n, (r, t, e) in enumerate(units):
            if n + LA < len(units):
                q.append(mm1(*units[n + LA]))
            yield
            bb = q.pop(0)
            gs = []
            for k in range(L // 16):
                b = bb[k * 16:(k + 1) * 16]
                th = jnp.tanh(b * (b * b + _KK))
                gs.append(b * th + b)
                yield
            gq.append((r, t, e, jnp.concatenate(gs, 0).astype(bf16)))
            if len(gq) > MD:
                mm2(*gq.pop(0))
            yield
        for u in gq:
            mm2(*u)

    def body(m, c):
        gen = stage_c(m)
        next(gen)
        for r in range(R):
            stage_a(m, r)
        for cb in range(CB):
            stage_b(m, cb, gen)
        for _ in gen:
            pass
        for r in range(R):
            for t in range(T):
                stage_ln(m, r, t)
        return c

    jax.lax.fori_loop(0, TH // R, body, 0)


@jax.jit
def pallas_standalone__modern_conv_block_replknet__vision_kernel(
    x: jax.Array,
    dw_large: jax.Array,
    dw_small: jax.Array,
    w1: jax.Array,
    w2: jax.Array,
):
    B, H, W, C = x.shape
    E = w1.shape[1]
    Kl, Ks = dw_large.shape[0], dw_small.shape[0]
    K = max(Kl, Ks)
    assert B == 1 and K <= 5 and H % TH == 0 and W % L == 0 and C % 16 == 0
    nb = H // TH
    xt = jnp.transpose(x.reshape(H, W, C), (0, 2, 1))
    full = lambda a: pl.BlockSpec(a.shape, lambda s: (0,) * a.ndim)
    w2t = w2.T
    out = pl.pallas_call(
        functools.partial(_kernel, C=C, W=W, E=E, K=K, Kl=Kl, Ks=Ks),
        grid=(nb + 1,),
        in_specs=[
            pl.BlockSpec((TH, C, W), lambda s: (jnp.minimum(s, nb - 1), 0, 0)),
            full(dw_large), full(dw_small), full(w1), full(w2t),
        ],
        out_specs=pl.BlockSpec((TH, C, W), lambda s: (jnp.maximum(s - 1, 0), 0, 0)),
        out_shape=jax.ShapeDtypeStruct((H, C, W), x.dtype),
        scratch_shapes=[
            pltpu.VMEM((NS, C, W), jnp.float32),
            pltpu.VMEM((K * K, C, L), jnp.float32),
            pltpu.VMEM((E // 2, C), jnp.uint32),
            pltpu.VMEM((C // 2, E), jnp.uint32),
            pltpu.VMEM((R, C // 2, W), jnp.uint32),
            pltpu.VMEM((R, C, W), jnp.float32),
        ],
        compiler_params=pltpu.CompilerParams(
            dimension_semantics=("arbitrary",),
            flags={"XLA_TPU_FORCE_LP_LLO_SCHEDULER": True},
            vmem_limit_bytes=64 * 1024 * 1024,
        ),
    )(xt, dw_large, dw_small, w1, w2t)
    return jnp.transpose(out, (0, 2, 1)).reshape(B, H, W, C)
```
